```python
import jax
import jax.numpy as jnp

def _softmax(x, axis=-1):
    return jax.nn.softmax(x, axis=axis)
def _gelu(x):
    return jax.nn.gelu(x, approximate=True)
def _silu(x):
    return jax.nn.silu(x)
def _sigmoid(x):
    return jax.nn.sigmoid(x)
def _layernorm(x, axis=-1, eps=1e-5):
    m = jnp.mean(x, axis=axis, keepdims=True)
    v = jnp.var(x, axis=axis, keepdims=True)
    return (x - m) / jnp.sqrt(v + eps)
def _scatter_add(tgt, idx, src, axis=0):
    return tgt.at[idx].add(src)
def _segment_sum(src, seg, n):
    return jax.ops.segment_sum(src, seg, n)
class _Rng:
    def __init__(self, key):
        self._k = key
    def _next(self):
        self._k, sub = jax.random.split(self._k)
        return sub
    def normal(self, shape):
        return jax.random.normal(self._next(), shape, dtype=jnp.bfloat16)
    def randint(self, lo, hi, shape):
        return jax.random.randint(self._next(), shape, lo, hi, dtype=jnp.int32)
    def uniform(self, shape, lo=0.0, hi=1.0):
        return jax.random.uniform(self._next(), shape, jnp.bfloat16, lo, hi)
    def permutation(self, n):
        return jax.random.permutation(self._next(), n)


kernel_name = 'sequential_preLN__linear_attn_block__moe_arch_mod__prompt'

def setup_inputs():
    _rng = _Rng(jax.random.key(int.from_bytes(__import__("os").urandom(4), "little")))
    _w = (lambda a: (lambda t: t.astype(jnp.bfloat16) if jnp.issubdtype(t.dtype, jnp.floating) else t)(jnp.asarray(a)))
    def _A_setup():
        B, S, D = 1, 2048, 1024
        return {
            "x": _w((lambda *s: _rng.normal(s) * 0.05)(B, S, D)),
            "wqkv": _w((lambda *s: _rng.normal(s) * 0.05)(D, 3 * D)),
            "wo": _w((lambda *s: _rng.normal(s) * 0.05)(D, D)),
        }
    _A_in = _A_setup()

    def _B_setup():
        B, S, D, F, C = 1, 2048, 1024, 3584, 2
        return {
            "x": _w((lambda *s: _rng.normal(s) * 0.05)(B, S, D)),
            "w_r": _w((lambda *s: _rng.normal(s) * 0.05)(D)),
            "w_gate": _w((lambda *s: _rng.normal(s) * 0.05)(D, F)),
            "w_up": _w((lambda *s: _rng.normal(s) * 0.05)(D, F)),
            "w_down": _w((lambda *s: _rng.normal(s) * 0.05)(F, D)),
        }
    _B_in = _B_setup()

    return {
        "A_x": _A_in["x"],
        "A_wqkv": _A_in["wqkv"],
        "A_wo": _A_in["wo"],
        "B_x": _B_in["x"],
        "B_w_r": _B_in["w_r"],
        "B_w_gate": _B_in["w_gate"],
        "B_w_up": _B_in["w_up"],
        "B_w_down": _B_in["w_down"],
    }

def reference(A_x, A_wqkv, A_wo, B_x, B_w_r, B_w_gate, B_w_up, B_w_down):
    def _A_ref(x, wqkv, wo):
        B, S, D = x.shape
        H = 32; Dh = D // H
        qkv = (lambda x, *d: x.transpose(*d))((x @ wqkv).reshape(B, S, 3, H, Dh), 2, 0, 3, 1, 4)
        q, k, v = qkv[0], qkv[1], qkv[2]
        phi = lambda t: jnp.where(t > 0, t + 1, jnp.exp(t)) + 1e-6
        pq, pk = phi(q), phi(k)
        kv = jnp.einsum("bhsd,bhse->bhde", pk, v)
        z = jnp.einsum("bhsd->bhd", pk)
        num = jnp.einsum("bhqd,bhde->bhqe", pq, kv)
        den = jnp.einsum("bhqd,bhd->bhq", pq, z)[..., None] + 1e-6
        o = num / den
        return (lambda x, *d: x.transpose(*d))(o, 0, 2, 1, 3).reshape(B, S, D) @ wo

    def _B_ref(x, w_r, w_gate, w_up, w_down):
        B, S, D = x.shape
        C = 2
        r = x @ w_r
        idx = jnp.argsort(-r, axis=-1)[:, :C]
        idx_e = jnp.repeat(idx.reshape(B, C, 1), D, axis=2)
        x_sel = jnp.take_along_axis(x, idx_e, axis=1)
        g = _silu(x_sel @ w_gate)
        u = x_sel @ w_up
        y = (g * u) @ w_down
        r_sel = _sigmoid(jnp.take_along_axis(r, idx, axis=1))
        y = y * r_sel.reshape(B, C, 1)
        b_off = (jnp.arange(B) * S).reshape(B, 1)
        flat_idx = (idx + b_off).reshape(B * C)
        zero = (x * 0.0).reshape(B * S, D)
        upd = _scatter_add(zero, flat_idx, y.reshape(B * C, D), axis=0)
        return x + upd.reshape(B, S, D)

    x = A_x
    h = x + _A_ref(_layernorm(x, axis=-1), A_wqkv, A_wo)
    h2 = h + _B_ref(_layernorm(h, axis=-1), B_w_r, B_w_gate, B_w_up, B_w_down)
    return h2
```

```python
import functools
import jax
import jax.numpy as jnp
from jax import lax
import jax.experimental.pallas as pl
import jax.experimental.pallas.tpu as pltpu

S, D, F, DH = 2048, 1024, 3584, 32
TS = 256
NT = S // TS
NG = D // 128
CW = 256
EPS = 1e-5
f32, bf16 = jnp.float32, jnp.bfloat16


def _ln(xf):
    mu = jnp.mean(xf, axis=-1, keepdims=True)
    d = xf - mu
    var = jnp.mean(d * d, axis=-1, keepdims=True)
    return d * lax.rsqrt(var + EPS)


def _phi(t):
    return jnp.where(t > 0, t + 1.0, jnp.exp(t)) + 1e-6


def _dot(a, b):
    return jnp.dot(a, b, preferred_element_type=f32)


def _kernel(x_hbm, wqkv_hbm, wo_hbm, wr_ref, wg_hbm, wu_hbm, wd_hbm, out_hbm,
            x_v, wq_v, wk_v, wv_v, wo_v, wg_v, wu_v, wd_v, ln_v, out_v, kv_v, z_v, wp_v, zx_v, pq_v, h_v,
            xsem, wsem, osem):
    def xcopy(i):
        r = pl.ds(pl.multiple_of(i * TS, TS), TS)
        return pltpu.make_async_copy(x_hbm.at[r], x_v.at[r], xsem.at[i])

    def ocopy(i):
        r = pl.ds(pl.multiple_of(i * TS, TS), TS)
        return pltpu.make_async_copy(out_v.at[r], out_hbm.at[r], osem.at[i])

    cq = pltpu.make_async_copy(wqkv_hbm.at[:, pl.ds(0, D)], wq_v, wsem.at[0])
    ck = pltpu.make_async_copy(wqkv_hbm.at[:, pl.ds(D, D)], wk_v, wsem.at[1])
    cv = pltpu.make_async_copy(wqkv_hbm.at[:, pl.ds(2 * D, D)], wv_v, wsem.at[2])
    co = pltpu.make_async_copy(wo_hbm, wo_v, wsem.at[3])
    cg = pltpu.make_async_copy(wg_hbm, wg_v, wsem.at[4])
    cu = pltpu.make_async_copy(wu_hbm, wu_v, wsem.at[5])
    cd = pltpu.make_async_copy(wd_hbm, wd_v, wsem.at[6])

    xcopy(0).start()
    ck.start()
    cv.start()
    xcopy(1).start()
    kv_v[...] = jnp.zeros_like(kv_v)
    z_v[...] = jnp.zeros_like(z_v)

    def p1(i, carry):
        @pl.when(i + 2 < NT)
        def _():
            xcopy(i + 2).start()

        @pl.when(i == 0)
        def _():
            ck.wait()
            cv.wait()
            cq.start()

        @pl.when(i == 1)
        def _():
            co.start()

        @pl.when(i == 2)
        def _():
            cg.start()

        @pl.when(i == 4)
        def _():
            cu.start()

        @pl.when(i == 6)
        def _():
            cd.start()

        xcopy(i).wait()
        r = pl.ds(pl.multiple_of(i * TS, TS), TS)
        ln = _ln(x_v[r, :].astype(f32)).astype(bf16)
        ln_v[r, :] = ln
        for c in range(D // CW):
            cs = slice(c * CW, (c + 1) * CW)
            pk = _phi(_dot(ln, wk_v[:, cs]))
            v = _dot(ln, wv_v[:, cs]).astype(bf16)
            z_v[:, cs] += jnp.sum(pk.reshape(TS // 8, 8, CW), axis=0)
            pkb = pk.astype(bf16)
            for g in range(CW // 128):
                gs = slice(g * 128, (g + 1) * 128)
                G = c * (CW // 128) + g
                kv_v[G * 128:(G + 1) * 128, :] += lax.dot_general(
                    pkb[:, gs], v[:, gs], (((0,), (0,)), ((), ())), preferred_element_type=f32)
        return carry

    lax.fori_loop(0, NT, p1, 0)

    cq.wait()
    co.wait()
    ri = lax.broadcasted_iota(jnp.int32, (128, 128), 0) // DH
    ci = lax.broadcasted_iota(jnp.int32, (128, 128), 1) // DH
    bd = ri == ci
    z = jnp.sum(z_v[...], axis=0, keepdims=True)
    for g in range(NG):
        gs = slice(g * 128, (g + 1) * 128)
        kvm = jnp.where(bd, kv_v[gs, :], 0.0).astype(bf16)
        wp_v[gs, :] = _dot(kvm, wo_v[gs, :]).astype(bf16)
        zt = jnp.where(bd, jnp.broadcast_to(z[:, gs], (128, 128)), 0.0)
        zx_v[gs, :] = zt.T.astype(bf16)

    wr = wr_ref[...].astype(f32)
    sub = lax.broadcasted_iota(jnp.int32, (8, 1), 0)

    def p3(i, carry):
        m1, i1, m2, i2 = carry
        r = pl.ds(pl.multiple_of(i * TS, TS), TS)
        ln = ln_v[r, :]
        for c in range(D // CW):
            cs = slice(c * CW, (c + 1) * CW)
            pq = _phi(_dot(ln, wq_v[:, cs]))
            pqb = pq.astype(bf16)
            for g in range(CW // 128):
                gs = slice(g * 128, (g + 1) * 128)
                G = c * (CW // 128) + g
                den = _dot(pqb[:, gs], zx_v[G * 128:(G + 1) * 128, :]) + 1e-6
                pq_v[:, G * 128:(G + 1) * 128] = (pq[:, gs] / den).astype(bf16)
        pqn = pq_v[...]
        for c in range(D // CW):
            cs = slice(c * CW, (c + 1) * CW)
            h_v[:, cs] = x_v[r, cs].astype(f32) + _dot(pqn, wp_v[:, cs])
        h = h_v[...]
        l2 = _ln(h)
        ln_v[r, :] = l2.astype(bf16)
        out_v[r, :] = (h + l2).astype(bf16)
        ocopy(i).start()
        rr = jnp.sum(l2 * wr, axis=-1, keepdims=True)
        for j in range(TS // 8):
            rj = rr[8 * j:8 * j + 8]
            idx = sub + (i * TS + 8 * j)
            g1 = rj > m1
            g2 = rj > m2
            m2 = jnp.where(g1, m1, jnp.where(g2, rj, m2))
            i2 = jnp.where(g1, i1, jnp.where(g2, idx, i2))
            m1 = jnp.where(g1, rj, m1)
            i1 = jnp.where(g1, idx, i1)
        return m1, i1, m2, i2

    ninf = jnp.full((8, 1), -jnp.inf, f32)
    zi = jnp.zeros((8, 1), jnp.int32)
    m1, i1, m2, i2 = lax.fori_loop(0, NT, p3, (ninf, zi, ninf, zi))

    big = jnp.int32(S)
    a = jnp.max(m1)
    ia = jnp.min(jnp.where(m1 == a, i1, big))
    won = i1 == ia
    m1b = jnp.where(won, m2, m1)
    i1b = jnp.where(won, i2, i1)
    b = jnp.max(m1b)
    ib = jnp.min(jnp.where(m1b == b, i1b, big))
    ia = jnp.clip(ia, 0, S - 1)
    ib = jnp.clip(ib, 0, S - 1)

    ba = pl.multiple_of((ia // 16) * 16, 16)
    bb = pl.multiple_of((ib // 16) * 16, 16)
    row16 = lax.broadcasted_iota(jnp.int32, (16, 1), 0)
    xa = jnp.sum(jnp.where(row16 == ia - ba, ln_v[pl.ds(ba, 16), :].astype(f32), 0.0), axis=0, keepdims=True)
    xb = jnp.sum(jnp.where(row16 == ib - bb, ln_v[pl.ds(bb, 16), :].astype(f32), 0.0), axis=0, keepdims=True)
    xs = jnp.where(row16 == 0, xa, jnp.where(row16 == 1, xb, 0.0)).astype(bf16)
    cg.wait()
    cu.wait()
    cd.wait()
    gg = _dot(xs, wg_v[...])
    uu = _dot(xs, wu_v[...])
    act = (gg * jax.nn.sigmoid(gg) * uu).astype(bf16)
    y = _dot(act, wd_v[...])
    ya = y[0:1] * jax.nn.sigmoid(jnp.full((1, 1), a, f32))
    yb = y[1:2] * jax.nn.sigmoid(jnp.full((1, 1), b, f32))
    for i in range(NT):
        ocopy(i).wait()
    blk = out_v[pl.ds(ba, 16), :].astype(f32)
    out_v[pl.ds(ba, 16), :] = jnp.where(row16 == ia - ba, blk + ya, blk).astype(bf16)
    blk = out_v[pl.ds(bb, 16), :].astype(f32)
    out_v[pl.ds(bb, 16), :] = jnp.where(row16 == ib - bb, blk + yb, blk).astype(bf16)
    c1 = pltpu.make_async_copy(out_v.at[pl.ds(ba, 16)], out_hbm.at[pl.ds(ba, 16)], osem.at[0])
    c1.start()

    @pl.when(ba != bb)
    def _():
        c2 = pltpu.make_async_copy(out_v.at[pl.ds(bb, 16)], out_hbm.at[pl.ds(bb, 16)], osem.at[1])
        c2.start()
        c2.wait()
    c1.wait()


@jax.jit
def pallas_sequential_preLN__linear_attn_block__moe_arch_mod__prompt_kernel(
    A_x, A_wqkv, A_wo, B_x, B_w_r, B_w_gate, B_w_up, B_w_down,
):
    x2 = A_x.reshape(S, D)
    wr = B_w_r.reshape(1, D)
    hbm = pl.BlockSpec(memory_space=pl.ANY)
    out = pl.pallas_call(
        _kernel,
        out_shape=jax.ShapeDtypeStruct((S, D), bf16),
        in_specs=[hbm, hbm, hbm, pl.BlockSpec(memory_space=pltpu.VMEM), hbm, hbm, hbm],
        out_specs=hbm,
        scratch_shapes=[
            pltpu.VMEM((S, D), bf16),
            pltpu.VMEM((D, D), bf16),
            pltpu.VMEM((D, D), bf16),
            pltpu.VMEM((D, D), bf16),
            pltpu.VMEM((D, D), bf16),
            pltpu.VMEM((D, F), bf16),
            pltpu.VMEM((D, F), bf16),
            pltpu.VMEM((F, D), bf16),
            pltpu.VMEM((S, D), bf16),
            pltpu.VMEM((S, D), bf16),
            pltpu.VMEM((D, 128), f32),
            pltpu.VMEM((8, D), f32),
            pltpu.VMEM((D, D), bf16),
            pltpu.VMEM((D, 128), bf16),
            pltpu.VMEM((TS, D), bf16),
            pltpu.VMEM((TS, D), f32),
            pltpu.SemaphoreType.DMA((NT,)),
            pltpu.SemaphoreType.DMA((8,)),
            pltpu.SemaphoreType.DMA((NT,)),
        ],
        compiler_params=pltpu.CompilerParams(vmem_limit_bytes=100 * 1024 * 1024),
    )(x2, A_wqkv, A_wo, wr, B_w_gate, B_w_up, B_w_down)
    return out.reshape(1, S, D)
```

```python
import jax
import jax.numpy as jnp
from jax import lax
import jax.experimental.pallas as pl
import jax.experimental.pallas.tpu as pltpu

S, D, F, DH = 2048, 1024, 3584, 32
TS = 256
NT = S // TS
NG = D // 128
CW = 256
NC = D // CW
NP = 2 * NC
PRO = {6: (0, 1, 2, 3), 7: (4, 5, 6, 7)}
SIDE = ((0,), (1,), (2,), (3,), (4, 5), (6,), (7,), ())
EPS = 1e-5
f32, bf16 = jnp.float32, jnp.bfloat16


def _ln(xf):
    mu = jnp.mean(xf, axis=-1, keepdims=True)
    d = xf - mu
    var = jnp.mean(d * d, axis=-1, keepdims=True)
    return d * lax.rsqrt(var + EPS)


def _phi(t):
    return jnp.where(t > 0, t + 1.0, jnp.exp(t)) + 1e-6


def _dot(a, b):
    return jnp.dot(a, b, preferred_element_type=f32)


def _recip(d):
    r = pl.reciprocal(d, approx=True)
    return r * (2.0 - d * r)


def _kernel(x_hbm, wqkv_hbm, wo_hbm, wr_hbm, wg_hbm, wu_hbm, wd_hbm, out_hbm,
            x_v, wq_v, wk_v, wv_v, wo_v, wg_v, wu_v, wd_v, ln1_v, ln2_v, out_v, kv_v, z_v, wp_v, zx_v,
            lnA, lnB, pqA, pqB, hA, hB, pkt_s, v_s, wr_ref, zs,
            xsem, wsem, ksem, vsem, osem):
    def rows(t):
        if isinstance(t, int):
            return pl.ds(t * TS, TS)
        return pl.ds(pl.multiple_of(t * TS, TS), TS)

    def xcopy(t):
        return pltpu.make_async_copy(x_hbm.at[rows(t)], x_v.at[rows(t)], xsem.at[t])

    def ocopy(t):
        return pltpu.make_async_copy(out_v.at[rows(t)], out_hbm.at[rows(t)], osem.at[t])

    def ck(c):
        return pltpu.make_async_copy(wqkv_hbm.at[:, pl.ds(D + c * CW, CW)], wk_v.at[:, pl.ds(c * CW, CW)], ksem.at[c])

    def cv(c):
        return pltpu.make_async_copy(wqkv_hbm.at[:, pl.ds(2 * D + c * CW, CW)], wv_v.at[:, pl.ds(c * CW, CW)], vsem.at[c])

    cq = pltpu.make_async_copy(wqkv_hbm.at[:, pl.ds(0, D)], wq_v, wsem.at[0])
    co = pltpu.make_async_copy(wo_hbm, wo_v, wsem.at[3])
    cg = pltpu.make_async_copy(wg_hbm, wg_v, wsem.at[4])
    cu = pltpu.make_async_copy(wu_hbm, wu_v, wsem.at[5])
    cd = pltpu.make_async_copy(wd_hbm, wd_v, wsem.at[6])

    def prow(t, p, n):
        h = TS // n
        if isinstance(t, int):
            return pl.ds(t * TS + p * h, h)
        return pl.ds(pl.multiple_of(t * TS + p * h, h), h)

    def ln1_piece(t, dst, p, n=NP):
        h = TS // n
        ln = _ln(x_v[prow(t, p, n), :].astype(f32)).astype(bf16)
        dst[p * h:(p + 1) * h, :] = ln
        ln1_v[prow(t, p, n), :] = ln

    cr = pltpu.make_async_copy(wr_hbm, wr_ref, wsem.at[7])

    def anchor(val, refs, extra=None):
        zero = zs[0]
        u = None
        for ref in refs:
            w = pltpu.bitcast(ref[pl.ds(pl.multiple_of(zero, 16), 16), 0:128], jnp.int32)
            u = w if u is None else u & w
        if extra is not None:
            u = u & extra
        u = u & zero
        n = 8 * 4 // val.dtype.itemsize
        v0 = pltpu.bitcast(pltpu.bitcast(val[0:n, 0:128], jnp.int32) | u, val.dtype)
        left = jnp.concatenate([v0, val[n:, 0:128]], axis=0)
        return jnp.concatenate([left, val[:, 128:]], axis=1)

    def ln1_step(t, dst):
        ln1_piece(t, dst, 0, 1)

    def kv_flush(c):
        for g in range(CW // 128):
            gs = slice(g * 128, (g + 1) * 128)
            G = c * (CW // 128) + g
            kv_v[G * 128:(G + 1) * 128, :] += _dot(pkt_s[gs, :], v_s[:, gs])

    def kv_chunk(src, c, side=None, dst=None, first=False, mid=None):
        cs = slice(c * CW, (c + 1) * CW)
        k = _dot(src[...], wk_v[:, cs])
        if side is not None and c > 0 and first is not None:
            k = anchor(k, (dst,))
        if not first:
            kv_flush((c - 1) % NC)
        pk = _phi(k)
        if side is not None:
            side(2 * c)
        if mid is not None:
            mid()
        v = _dot(src[...], wv_v[:, cs])
        if side is not None:
            side(2 * c + 1)
        z_v[:, cs] += jnp.sum(pk.reshape(TS // 8, 8, CW), axis=0)
        for g in range(CW // 128):
            gs = slice(g * 128, (g + 1) * 128)
            pkt_s[gs, :] = pk[:, gs].T.astype(bf16)
        v_s[...] = v.astype(bf16)

    def kv_step(src, side=None, dst=None):
        for c in range(NC):
            kv_chunk(src, c, side, dst)

    xcopy(0).start()
    ck(0).start()
    cv(0).start()
    kv_v[...] = jnp.zeros_like(kv_v)
    z_v[...] = jnp.zeros_like(z_v)
    nxt = [ck(1), cv(1), ck(2), cv(2), xcopy(1), ck(3), cv(3)]
    xcopy(0).wait()
    nxt.pop(0).start()
    sgn = jnp.max(pltpu.bitcast(x_v[0:16, 0:128], jnp.int32)) >> 31
    zs[0] = sgn & (sgn ^ -1)
    ln1_step(0, lnA)

    def gate(cp):
        def f():
            cp.wait()
            if nxt:
                nxt.pop(0).start()
                if len(nxt) == 0:
                    for t in range(2, NT):
                        xcopy(t).start()
                    for w in (cr, cq, co, cg, cu, cd):
                        w.start()
        return f

    for c in range(NC):
        gate(ck(c))()
        if c == NC - 1:
            xcopy(1).wait()
        kv_chunk(lnA, c, None if c < NC - 1 else (lambda p: [ln1_piece(1, lnB, q) for q in PRO[p]]), lnB,
                 first=(True if c == 0 else None), mid=gate(cv(c)))

    def p1(j, carry):
        t = 2 * j + 1
        xcopy(t + 1).wait()

        kv_step(lnB, lambda p: ln1_piece(t + 1, lnA, p), lnA)

        xcopy(t + 2).wait()
        kv_step(lnA, lambda p: ln1_piece(t + 2, lnB, p), lnB)
        return carry

    lax.fori_loop(0, (NT - 2) // 2, p1, 0)
    kv_step(lnB)
    kv_flush(NC - 1)

    cq.wait()
    cr.wait()
    co.wait()
    ri = lax.broadcasted_iota(jnp.int32, (128, 128), 0) // DH
    ci = lax.broadcasted_iota(jnp.int32, (128, 128), 1) // DH
    bd = ri == ci
    z = jnp.sum(z_v[...], axis=0, keepdims=True)
    for g in range(NG):
        gs = slice(g * 128, (g + 1) * 128)
        zt = jnp.where(bd, jnp.broadcast_to(z[:, gs], (128, 128)), 0.0)
        zx_v[gs, :] = zt.T.astype(bf16)
    for g in range(NG):
        gs = slice(g * 128, (g + 1) * 128)
        kvm = jnp.where(bd, kv_v[gs, :], 0.0).astype(bf16)
        wp_v[gs, :] = _dot(kvm, wo_v[gs, :]).astype(bf16)

    wr = wr_ref[...].reshape(1, D).astype(f32)
    sub = lax.broadcasted_iota(jnp.int32, (8, 1), 0)

    def attn_step(t, pq_v, h_v, side=None):
        r = rows(t)
        for c in range(NC):
            cs = slice(c * CW, (c + 1) * CW)
            q = _dot(ln1_v[r, :], wq_v[:, cs])
            if side is not None and c > 0 and SIDE[c - 1]:
                q = anchor(q, (ln2_v, out_v), side(None))
            if side is not None:
                for p in SIDE[c]:
                    side(p)
            pq = _phi(q)
            pqb = pq.astype(bf16)
            for g in range(CW // 128):
                gs = slice(g * 128, (g + 1) * 128)
                G = c * (CW // 128) + g
                den = _dot(pqb[:, gs], zx_v[G * 128:(G + 1) * 128, :]) + 1e-6
                pq_v[:, G * 128:(G + 1) * 128] = (pq[:, gs] * _recip(den)).astype(bf16)
        for c in range(NC):
            cs = slice(c * CW, (c + 1) * CW)
            lhs = pq_v[...]
            if side is not None and SIDE[NC + c - 1]:
                lhs = anchor(lhs, (ln2_v, out_v), side(None))
            h_v[:, cs] = x_v[r, cs].astype(f32) + _dot(lhs, wp_v[:, cs])
            if side is not None:
                for p in SIDE[NC + c]:
                    side(p)

    def ln2_piece(t, h_v, carry, p, n=NP):
        m1, i1, m2, i2 = carry
        hh = TS // n
        r = prow(t, p, n)
        h = h_v[p * hh:(p + 1) * hh, :]
        l2 = _ln(h)
        ln2_v[r, :] = l2.astype(bf16)
        out_v[r, :] = (h + l2).astype(bf16)
        rr = jnp.sum(l2 * wr, axis=-1, keepdims=True)
        for k in range(hh // 8):
            rj = rr[8 * k:8 * k + 8]
            idx = sub + (t * TS + p * hh + 8 * k)
            g1 = rj > m1
            g2 = rj > m2
            m2 = jnp.where(g1, m1, jnp.where(g2, rj, m2))
            i2 = jnp.where(g1, i1, jnp.where(g2, idx, i2))
            m1 = jnp.where(g1, rj, m1)
            i1 = jnp.where(g1, idx, i1)
        return m1, i1, m2, i2

    def ln2_step(t, h_v, carry):
        return ln2_piece(t, h_v, carry, 0, 1)

    def both(t, pq_v, h_v, hprev, carry):
        box = [carry]

        def side(p):
            if p is None:
                return box[0][3]
            box[0] = ln2_piece(t - 1, hprev, box[0], p)
        attn_step(t, pq_v, h_v, side)
        return box[0]

    ninf = jnp.full((8, 1), -jnp.inf, f32)
    zi = jnp.zeros((8, 1), jnp.int32)
    carry = (ninf, zi, ninf, zi)
    attn_step(0, pqA, hA)

    def p3(j, carry):
        t = 2 * j + 1
        carry = both(t, pqB, hB, hA, carry)
        ocopy(t - 1).start()
        carry = both(t + 1, pqA, hA, hB, carry)
        ocopy(t).start()
        return carry

    carry = lax.fori_loop(0, (NT - 2) // 2, p3, carry)
    carry = both(NT - 1, pqB, hB, hA, carry)
    ocopy(NT - 2).start()
    m1, i1, m2, i2 = ln2_step(NT - 1, hB, carry)
    ocopy(NT - 1).start()

    big = jnp.int32(S)
    a = jnp.max(m1, axis=0, keepdims=True)
    ia = jnp.min(jnp.where(m1 == a, i1, big), axis=0, keepdims=True)
    won = i1 == ia
    m1b = jnp.where(won, m2, m1)
    i1b = jnp.where(won, i2, i1)
    b = jnp.max(m1b, axis=0, keepdims=True)
    ib = jnp.min(jnp.where(m1b == b, i1b, big), axis=0, keepdims=True)
    ia = jnp.clip(ia[0, 0], 0, S - 1)
    ib = jnp.clip(ib[0, 0], 0, S - 1)

    ba = pl.multiple_of((ia // 16) * 16, 16)
    bb = pl.multiple_of((ib // 16) * 16, 16)
    row16 = lax.broadcasted_iota(jnp.int32, (16, 1), 0)
    ma = row16 == ia - ba
    mb = row16 == ib - bb
    xa = jnp.sum(jnp.where(ma, ln2_v[pl.ds(ba, 16), :].astype(f32), 0.0), axis=0, keepdims=True)
    xb = jnp.sum(jnp.where(mb, ln2_v[pl.ds(bb, 16), :].astype(f32), 0.0), axis=0, keepdims=True)
    xs = jnp.where(row16 == 0, xa, jnp.where(row16 == 1, xb, 0.0)).astype(bf16)
    cg.wait()
    cu.wait()
    cd.wait()
    gg = _dot(xs, wg_v[...])
    uu = _dot(xs, wu_v[...])
    act = (gg * jax.nn.sigmoid(gg) * uu).astype(bf16)
    y = jnp.zeros((16, D), f32)
    for k in range(F // 256):
        y = y + _dot(act[:, k * 256:(k + 1) * 256], wd_v[k * 256:(k + 1) * 256, :])
    ya = y[0:1] * jax.nn.sigmoid(a)
    yb = y[1:2] * jax.nn.sigmoid(b)
    for i in range(NT):
        ocopy(i).wait()
    blk = out_v[pl.ds(ba, 16), :].astype(f32)
    out_v[pl.ds(ba, 16), :] = jnp.where(ma, blk + ya, blk).astype(bf16)
    blk = out_v[pl.ds(bb, 16), :].astype(f32)
    out_v[pl.ds(bb, 16), :] = jnp.where(mb, blk + yb, blk).astype(bf16)
    c1 = pltpu.make_async_copy(out_v.at[pl.ds(ba, 16)], out_hbm.at[pl.ds(ba, 16)], osem.at[0])
    c1.start()

    @pl.when(ba != bb)
    def _():
        c2 = pltpu.make_async_copy(out_v.at[pl.ds(bb, 16)], out_hbm.at[pl.ds(bb, 16)], osem.at[1])
        c2.start()
        c2.wait()
    c1.wait()


@jax.jit
def pallas_sequential_preLN__linear_attn_block__moe_arch_mod__prompt_kernel(
    A_x, A_wqkv, A_wo, B_x, B_w_r, B_w_gate, B_w_up, B_w_down,
):
    x2 = A_x.reshape(S, D)
    hbm = pl.BlockSpec(memory_space=pl.ANY)
    out = pl.pallas_call(
        _kernel,
        out_shape=jax.ShapeDtypeStruct((S, D), bf16),
        in_specs=[hbm] * 7,
        out_specs=hbm,
        scratch_shapes=[
            pltpu.VMEM((S, D), bf16),
            pltpu.VMEM((D, D), bf16),
            pltpu.VMEM((D, D), bf16),
            pltpu.VMEM((D, D), bf16),
            pltpu.VMEM((D, D), bf16),
            pltpu.VMEM((D, F), bf16),
            pltpu.VMEM((D, F), bf16),
            pltpu.VMEM((F, D), bf16),
            pltpu.VMEM((S, D), bf16),
            pltpu.VMEM((S, D), bf16),
            pltpu.VMEM((S, D), bf16),
            pltpu.VMEM((D, 128), f32),
            pltpu.VMEM((8, D), f32),
            pltpu.VMEM((D, D), bf16),
            pltpu.VMEM((D, 128), bf16),
            pltpu.VMEM((TS, D), bf16),
            pltpu.VMEM((TS, D), bf16),
            pltpu.VMEM((TS, D), bf16),
            pltpu.VMEM((TS, D), bf16),
            pltpu.VMEM((TS, D), f32),
            pltpu.VMEM((TS, D), f32),
            pltpu.VMEM((CW, TS), bf16),
            pltpu.VMEM((TS, CW), bf16),
            pltpu.VMEM((D,), bf16),
            pltpu.SMEM((1,), jnp.int32),
            pltpu.SemaphoreType.DMA((NT,)),
            pltpu.SemaphoreType.DMA((8,)),
            pltpu.SemaphoreType.DMA((NC,)),
            pltpu.SemaphoreType.DMA((NC,)),
            pltpu.SemaphoreType.DMA((NT,)),
        ],
        compiler_params=pltpu.CompilerParams(vmem_limit_bytes=100 * 1024 * 1024),
    )(x2, A_wqkv, A_wo, B_w_r, B_w_gate, B_w_up, B_w_down)
    return out.reshape(1, S, D)
```

```python
import jax
import jax.numpy as jnp
from jax import lax
import jax.experimental.pallas as pl
import jax.experimental.pallas.tpu as pltpu

S, D, F, DH = 2048, 1024, 3584, 32
TS = 256
NT = S // TS
NG = D // 128
CW = 256
NC = D // CW
NP = 2 * NC
PRO = {6: (0, 1, 2, 3), 7: (4, 5, 6, 7)}
SIDE = ((0,), (1,), (2,), (3,), (4, 5), (6,), (7,), ())
EPS = 1e-5
f32, bf16 = jnp.float32, jnp.bfloat16


def _ln(xf):
    mu = jnp.mean(xf, axis=-1, keepdims=True)
    d = xf - mu
    var = jnp.mean(d * d, axis=-1, keepdims=True)
    return d * lax.rsqrt(var + EPS)


def _phi(t):
    return jnp.where(t > 0, t + 1.0, jnp.exp(t)) + 1e-6


def _dot(a, b):
    return jnp.dot(a, b, preferred_element_type=f32)


def _recip(d):
    r = pl.reciprocal(d, approx=True)
    return r * (2.0 - d * r)


def _kernel(x_hbm, wqkv_hbm, wo_hbm, wr_hbm, wg_hbm, wu_hbm, wd_hbm, out_hbm,
            x_v, wq_v, wk_v, wv_v, wo_v, wg_v, wu_v, wd_v, ln1_v, ln2_v, out_v, acc_v, z_v, wp_v, zx_v,
            lnA, lnB, pqA, pqB, hA, hB, pktA, pktB, wr_ref, zs,
            xsem, wsem, ksem, osem):
    def rows(t):
        if isinstance(t, int):
            return pl.ds(t * TS, TS)
        return pl.ds(pl.multiple_of(t * TS, TS), TS)

    def xcopy(t):
        return pltpu.make_async_copy(x_hbm.at[rows(t)], x_v.at[rows(t)], xsem.at[t])

    def ocopy(t):
        return pltpu.make_async_copy(out_v.at[rows(t)], out_hbm.at[rows(t)], osem.at[t])

    def ck(c):
        return pltpu.make_async_copy(wqkv_hbm.at[:, pl.ds(D + c * CW, CW)], wk_v.at[:, pl.ds(c * CW, CW)], ksem.at[c])

    cv = pltpu.make_async_copy(wqkv_hbm.at[:, pl.ds(2 * D, D)], wv_v, wsem.at[2])
    cq = pltpu.make_async_copy(wqkv_hbm.at[:, pl.ds(0, D)], wq_v, wsem.at[0])
    co = pltpu.make_async_copy(wo_hbm, wo_v, wsem.at[3])
    cg = pltpu.make_async_copy(wg_hbm, wg_v, wsem.at[4])
    cu = pltpu.make_async_copy(wu_hbm, wu_v, wsem.at[5])
    cd = pltpu.make_async_copy(wd_hbm, wd_v, wsem.at[6])

    def prow(t, p, n):
        h = TS // n
        if isinstance(t, int):
            return pl.ds(t * TS + p * h, h)
        return pl.ds(pl.multiple_of(t * TS + p * h, h), h)

    def ln1_piece(t, dst, p, n=NP):
        h = TS // n
        ln = _ln(x_v[prow(t, p, n), :].astype(f32)).astype(bf16)
        dst[p * h:(p + 1) * h, :] = ln

    cr = pltpu.make_async_copy(wr_hbm, wr_ref, wsem.at[7])

    def anchor(val, refs, extra=None):
        zero = zs[0]
        u = None
        for ref in refs:
            w = pltpu.bitcast(ref[pl.ds(pl.multiple_of(zero, 16), 16), 0:128], jnp.int32)
            u = w if u is None else u & w
        if extra is not None:
            u = u & extra
        u = u & zero
        n = 8 * 4 // val.dtype.itemsize
        v0 = pltpu.bitcast(pltpu.bitcast(val[0:n, 0:128], jnp.int32) | u, val.dtype)
        left = jnp.concatenate([v0, val[n:, 0:128]], axis=0)
        return jnp.concatenate([left, val[:, 128:]], axis=1)

    def ln1_step(t, dst):
        ln1_piece(t, dst, 0, 1)

    def kv_chunk(pkt, src, c, side=None, dst=None, anch=True):
        cs = slice(c * CW, (c + 1) * CW)
        k = _dot(src[...], wk_v[:, cs])
        if side is not None and c > 0 and anch:
            k = anchor(k, (dst,))
        pk = _phi(k)
        if side is not None:
            side(2 * c)
            side(2 * c + 1)
        z_v[:, cs] += jnp.sum(pk.reshape(TS // 8, 8, CW), axis=0)
        for g in range(CW // 128):
            pkt[c * CW + g * 128:c * CW + (g + 1) * 128, :] = pk[:, g * 128:(g + 1) * 128].T.astype(bf16)

    def keep(t, src):
        return pltpu.make_async_copy(src, ln1_v.at[rows(t)], wsem.at[1])

    def m_part(t, pkt, c):
        cs = slice(c * CW, (c + 1) * CW)
        acc_v[:, cs] += _dot(pkt[...], ln1_v[rows(t), cs])

    def m_first(c):
        cs = slice(c * CW, (c + 1) * CW)
        acc_v[cs, :] = _dot(pktA[cs, :], lnA[...])

    def kv_step(t, src, pkt, pprev, side=None, dst=None):
        keep(t - 1, dst).wait()
        keep(t, src).start()
        for c in range(NC):
            kv_chunk(pkt, src, c, side, dst)
            m_part(t - 1, pprev, c)

    xcopy(0).start()
    ck(0).start()
    ck(1).start()
    z_v[...] = jnp.zeros_like(z_v)
    xcopy(0).wait()
    ck(2).start()
    sgn = jnp.max(pltpu.bitcast(x_v[0:16, 0:128], jnp.int32)) >> 31
    zs[0] = sgn & (sgn ^ -1)
    ln1_step(0, lnA)
    keep(0, lnA).start()
    for c in range(NC):
        ck(c).wait()
        if c == 0:
            xcopy(1).start()
        elif c == 1:
            ck(3).start()
        elif c == 2:
            xcopy(1).wait()
        else:
            for t in range(2, NT):
                xcopy(t).start()
            for w in (cv, cr, co, cq, cg, cu, cd):
                w.start()
        kv_chunk(pktA, lnA, c, None if c < 2 else (lambda p: [ln1_piece(1, lnB, 2 * p - 8 + q) for q in (0, 1)]), lnB, anch=(c == 3))
        if c > 0:
            m_first(c - 1)
    keep(0, lnA).wait()
    keep(1, lnB).start()
    m_first(NC - 1)
    xcopy(2).wait()
    for c in range(NC):
        kv_chunk(pktB, lnB, c, lambda p: ln1_piece(2, lnA, p), lnA)

    def p1(j, carry):
        t = 2 * j + 2
        xcopy(t + 1).wait()
        kv_step(t, lnA, pktA, pktB, lambda p: ln1_piece(t + 1, lnB, p), lnB)

        @pl.when(t + 2 < NT)
        def _():
            xcopy(t + 2).wait()
        nxt = jnp.minimum(t + 2, NT - 1)
        kv_step(t + 1, lnB, pktB, pktA, lambda p: ln1_piece(nxt, lnA, p), lnA)
        return carry

    lax.fori_loop(0, (NT - 2) // 2, p1, 0)
    keep(NT - 1, lnB).wait()
    for c in range(NC):
        m_part(NT - 1, pktB, c)

    cq.wait()
    cr.wait()
    cv.wait()
    co.wait()
    ri = lax.broadcasted_iota(jnp.int32, (128, 128), 0) // DH
    ci = lax.broadcasted_iota(jnp.int32, (128, 128), 1) // DH
    bd = ri == ci
    z = jnp.sum(z_v[...], axis=0, keepdims=True)
    for g in range(NG):
        gs = slice(g * 128, (g + 1) * 128)
        zt = jnp.where(bd, jnp.broadcast_to(z[:, gs], (128, 128)), 0.0)
        zx_v[gs, :] = zt.T.astype(bf16)
    for g in range(NG):
        gs = slice(g * 128, (g + 1) * 128)
        kvm = jnp.where(bd, _dot(acc_v[gs, :].astype(bf16), wv_v[:, gs]), 0.0).astype(bf16)
        wp_v[gs, :] = _dot(kvm, wo_v[gs, :]).astype(bf16)

    wr = wr_ref[...].reshape(1, D).astype(f32)
    sub = lax.broadcasted_iota(jnp.int32, (8, 1), 0)

    def attn_step(t, pq_v, h_v, side=None):
        r = rows(t)
        for c in range(NC):
            cs = slice(c * CW, (c + 1) * CW)
            q = _dot(ln1_v[r, :], wq_v[:, cs])
            if side is not None and c > 0 and SIDE[c - 1]:
                q = anchor(q, (ln2_v, out_v), side(None))
            if side is not None:
                for p in SIDE[c]:
                    side(p)
            pq = _phi(q)
            pqb = pq.astype(bf16)
            for g in range(CW // 128):
                gs = slice(g * 128, (g + 1) * 128)
                G = c * (CW // 128) + g
                den = _dot(pqb[:, gs], zx_v[G * 128:(G + 1) * 128, :]) + 1e-6
                pq_v[:, G * 128:(G + 1) * 128] = (pq[:, gs] * _recip(den)).astype(bf16)
        for c in range(NC):
            cs = slice(c * CW, (c + 1) * CW)
            lhs = pq_v[...]
            if side is not None and SIDE[NC + c - 1]:
                lhs = anchor(lhs, (ln2_v, out_v), side(None))
            h_v[:, cs] = x_v[r, cs].astype(f32) + _dot(lhs, wp_v[:, cs])
            if side is not None:
                for p in SIDE[NC + c]:
                    side(p)

    def ln2_piece(t, h_v, carry, p, n=NP):
        m1, i1, m2, i2 = carry
        hh = TS // n
        r = prow(t, p, n)
        h = h_v[p * hh:(p + 1) * hh, :]
        l2 = _ln(h)
        ln2_v[r, :] = l2.astype(bf16)
        out_v[r, :] = (h + l2).astype(bf16)
        rr = jnp.sum(l2 * wr, axis=-1, keepdims=True)
        for k in range(hh // 8):
            rj = rr[8 * k:8 * k + 8]
            idx = sub + (t * TS + p * hh + 8 * k)
            g1 = rj > m1
            g2 = rj > m2
            m2 = jnp.where(g1, m1, jnp.where(g2, rj, m2))
            i2 = jnp.where(g1, i1, jnp.where(g2, idx, i2))
            m1 = jnp.where(g1, rj, m1)
            i1 = jnp.where(g1, idx, i1)
        return m1, i1, m2, i2

    def ln2_step(t, h_v, carry):
        return ln2_piece(t, h_v, carry, 0, 1)

    def both(t, pq_v, h_v, hprev, carry):
        box = [carry]

        def side(p):
            if p is None:
                return box[0][3]
            box[0] = ln2_piece(t - 1, hprev, box[0], p)
        attn_step(t, pq_v, h_v, side)
        return box[0]

    ninf = jnp.full((8, 1), -jnp.inf, f32)
    zi = jnp.zeros((8, 1), jnp.int32)
    carry = (ninf, zi, ninf, zi)
    attn_step(0, pqA, hA)

    def p3(j, carry):
        t = 2 * j + 1
        carry = both(t, pqB, hB, hA, carry)
        ocopy(t - 1).start()
        carry = both(t + 1, pqA, hA, hB, carry)
        ocopy(t).start()
        return carry

    carry = lax.fori_loop(0, (NT - 2) // 2, p3, carry)
    carry = both(NT - 1, pqB, hB, hA, carry)
    ocopy(NT - 2).start()
    m1, i1, m2, i2 = ln2_step(NT - 1, hB, carry)
    ocopy(NT - 1).start()

    big = jnp.int32(S)
    a = jnp.max(m1, axis=0, keepdims=True)
    ia = jnp.min(jnp.where(m1 == a, i1, big), axis=0, keepdims=True)
    won = i1 == ia
    m1b = jnp.where(won, m2, m1)
    i1b = jnp.where(won, i2, i1)
    b = jnp.max(m1b, axis=0, keepdims=True)
    ib = jnp.min(jnp.where(m1b == b, i1b, big), axis=0, keepdims=True)
    ia = jnp.clip(ia[0, 0], 0, S - 1)
    ib = jnp.clip(ib[0, 0], 0, S - 1)

    ba = pl.multiple_of((ia // 16) * 16, 16)
    bb = pl.multiple_of((ib // 16) * 16, 16)
    row16 = lax.broadcasted_iota(jnp.int32, (16, 1), 0)
    ma = row16 == ia - ba
    mb = row16 == ib - bb
    xa = jnp.sum(jnp.where(ma, ln2_v[pl.ds(ba, 16), :].astype(f32), 0.0), axis=0, keepdims=True)
    xb = jnp.sum(jnp.where(mb, ln2_v[pl.ds(bb, 16), :].astype(f32), 0.0), axis=0, keepdims=True)
    xs = jnp.where(row16 == 0, xa, jnp.where(row16 == 1, xb, 0.0)).astype(bf16)
    cg.wait()
    cu.wait()
    cd.wait()
    gg = _dot(xs, wg_v[...])
    uu = _dot(xs, wu_v[...])
    act = (gg * jax.nn.sigmoid(gg) * uu).astype(bf16)
    y = jnp.zeros((16, D), f32)
    for k in range(F // 256):
        y = y + _dot(act[:, k * 256:(k + 1) * 256], wd_v[k * 256:(k + 1) * 256, :])
    ya = y[0:1] * jax.nn.sigmoid(a)
    yb = y[1:2] * jax.nn.sigmoid(b)
    for i in range(NT):
        ocopy(i).wait()
    blk = out_v[pl.ds(ba, 16), :].astype(f32)
    out_v[pl.ds(ba, 16), :] = jnp.where(ma, blk + ya, blk).astype(bf16)
    blk = out_v[pl.ds(bb, 16), :].astype(f32)
    out_v[pl.ds(bb, 16), :] = jnp.where(mb, blk + yb, blk).astype(bf16)
    c1 = pltpu.make_async_copy(out_v.at[pl.ds(ba, 16)], out_hbm.at[pl.ds(ba, 16)], osem.at[0])
    c1.start()

    @pl.when(ba != bb)
    def _():
        c2 = pltpu.make_async_copy(out_v.at[pl.ds(bb, 16)], out_hbm.at[pl.ds(bb, 16)], osem.at[1])
        c2.start()
        c2.wait()
    c1.wait()


@jax.jit
def pallas_sequential_preLN__linear_attn_block__moe_arch_mod__prompt_kernel(
    A_x, A_wqkv, A_wo, B_x, B_w_r, B_w_gate, B_w_up, B_w_down,
):
    x2 = A_x.reshape(S, D)
    hbm = pl.BlockSpec(memory_space=pl.ANY)
    out = pl.pallas_call(
        _kernel,
        out_shape=jax.ShapeDtypeStruct((S, D), bf16),
        in_specs=[hbm] * 7,
        out_specs=hbm,
        scratch_shapes=[
            pltpu.VMEM((S, D), bf16),
            pltpu.VMEM((D, D), bf16),
            pltpu.VMEM((D, D), bf16),
            pltpu.VMEM((D, D), bf16),
            pltpu.VMEM((D, D), bf16),
            pltpu.VMEM((D, F), bf16),
            pltpu.VMEM((D, F), bf16),
            pltpu.VMEM((F, D), bf16),
            pltpu.VMEM((S, D), bf16),
            pltpu.VMEM((S, D), bf16),
            pltpu.VMEM((S, D), bf16),
            pltpu.VMEM((D, D), f32),
            pltpu.VMEM((8, D), f32),
            pltpu.VMEM((D, D), bf16),
            pltpu.VMEM((D, 128), bf16),
            pltpu.VMEM((TS, D), bf16),
            pltpu.VMEM((TS, D), bf16),
            pltpu.VMEM((TS, D), bf16),
            pltpu.VMEM((TS, D), bf16),
            pltpu.VMEM((TS, D), f32),
            pltpu.VMEM((TS, D), f32),
            pltpu.VMEM((D, TS), bf16),
            pltpu.VMEM((D, TS), bf16),
            pltpu.VMEM((D,), bf16),
            pltpu.SMEM((1,), jnp.int32),
            pltpu.SemaphoreType.DMA((NT,)),
            pltpu.SemaphoreType.DMA((8,)),
            pltpu.SemaphoreType.DMA((NC,)),
            pltpu.SemaphoreType.DMA((NT,)),
        ],
        compiler_params=pltpu.CompilerParams(vmem_limit_bytes=100 * 1024 * 1024),
    )(x2, A_wqkv, A_wo, B_w_r, B_w_gate, B_w_up, B_w_down)
    return out.reshape(1, S, D)
```
